```python
import os as _os
_os.environ.setdefault('JAX_PLATFORMS', 'cpu')
import jax
import jax.numpy as jnp

def _softmax(x, axis=-1):
    return jax.nn.softmax(x, axis=axis)

def _gelu(x):
    return jax.nn.gelu(x, approximate=True)

def _silu(x):
    return jax.nn.silu(x)

def _sigmoid(x):
    return jax.nn.sigmoid(x)

def _layernorm(x, axis=-1, eps=1e-05):
    m = jnp.mean(x, axis=axis, keepdims=True)
    v = jnp.var(x, axis=axis, keepdims=True)
    return (x - m) / jnp.sqrt(v + eps)

def _scatter_add(tgt, idx, src, axis=0):
    return tgt.at[idx].add(src)

def _segment_sum(src, seg, n):
    return jax.ops.segment_sum(src, seg, n)

class _Rng:

    def __init__(self, key):
        self._k = key

    def _next(self):
        self._k, sub = jax.random.split(self._k)
        return sub

    def normal(self, shape):
        return jax.random.normal(self._next(), shape, dtype=jnp.bfloat16)

    def randint(self, lo, hi, shape):
        return jax.random.randint(self._next(), shape, lo, hi, dtype=jnp.int32)

    def uniform(self, shape, lo=0.0, hi=1.0):
        return jax.random.uniform(self._next(), shape, jnp.bfloat16, lo, hi)

    def permutation(self, n):
        return jax.random.permutation(self._next(), n)
kernel_name = 'adaLN_cond__mha_block__geglu_ffn__prompt'

def setup_inputs():
    _rng = _Rng(jax.random.key(int.from_bytes(__import__("os").urandom(4), "little")))
    _w = lambda a: (lambda t: t.astype(jnp.bfloat16) if jnp.issubdtype(t.dtype, jnp.floating) else t)(jnp.asarray(a))

    def _A_setup():
        B, S, D, H = (1, 2048, 640, 32)
        return {'x': _w((lambda *s: _rng.normal(s) * 0.05)(B, S, D)), 'wqkv': _w((lambda *s: _rng.normal(s) * 0.05)(D, 3 * D)), 'wo': _w((lambda *s: _rng.normal(s) * 0.05)(D, D))}
    _A_in = _A_setup()

    def _B_setup():
        B, S, D, F = (1, 2048, 640, 1728)
        return {'x': _w((lambda *s: _rng.normal(s) * 0.05)(B, S, D)), 'w_gate': _w((lambda *s: _rng.normal(s) * 0.05)(D, F)), 'w_up': _w((lambda *s: _rng.normal(s) * 0.05)(D, F)), 'w_down': _w((lambda *s: _rng.normal(s) * 0.05)(F, D))}
    _B_in = _B_setup()
    return {'A_x': _A_in['x'], 'A_wqkv': _A_in['wqkv'], 'A_wo': _A_in['wo'], 'B_x': _B_in['x'], 'B_w_gate': _B_in['w_gate'], 'B_w_up': _B_in['w_up'], 'B_w_down': _B_in['w_down'], 'c': _w((lambda *s: _rng.normal(s) * 0.05)(1, 640) * 8.0), 'w_mod': _w((lambda *s: _rng.normal(s) * 0.05)(640, 6 * 640) * 640 ** (-0.5) * 8.0)}

def reference(A_x, A_wqkv, A_wo, B_x, B_w_gate, B_w_up, B_w_down, c, w_mod):

    def _A_ref(x, wqkv, wo):
        B, S, D = x.shape
        H = 32
        Dh = D // H
        qkv = (lambda x, *d: x.transpose(*d))((x @ wqkv).reshape(B, S, 3, H, Dh), 2, 0, 3, 1, 4)
        q, k, v = (qkv[0], qkv[1], qkv[2])
        scores = jnp.einsum('bhqd,bhkd->bhqk', q, k) * Dh ** (-0.5)
        p = _softmax(scores, axis=-1)
        o = jnp.einsum('bhqk,bhkd->bhqd', p, v)
        return (lambda x, *d: x.transpose(*d))(o, 0, 2, 1, 3).reshape(B, S, D) @ wo

    def _B_ref(x, w_gate, w_up, w_down):
        return _gelu(x @ w_gate) * (x @ w_up) @ w_down
    x = A_x
    mod = (_silu(c) @ w_mod).reshape(c.shape[0], 6, 1, -1)
    sa, ca, ga, sb, cb, gb = (mod[:, 0].copy(), mod[:, 1].copy(), mod[:, 2].copy(), mod[:, 3].copy(), mod[:, 4].copy(), mod[:, 5].copy())
    h = _layernorm(x, axis=-1) * (1 + ca) + sa
    x = x + ga * _A_ref(h, A_wqkv, A_wo)
    h = _layernorm(x, axis=-1) * (1 + cb) + sb
    x = x + gb * _B_ref(h, B_w_gate, B_w_up, B_w_down)
    return x
```

```python
import functools
import math

import jax
import jax.numpy as jnp
from jax import lax
import jax.experimental.pallas as pl
import jax.experimental.pallas.tpu as pltpu

S, D, H, DH, F = 2048, 640, 32, 20, 1728
LANES = 128
NT = D // LANES
QB = 512
KC = 128
NCH = S // KC
SKEW = 2
RB1 = 512
RB3 = 256
FMAIN = (F // LANES) * LANES
EPS = 1e-5
QSCALE = DH ** -0.5 * math.log2(math.e)
F32, BF16 = jnp.float32, jnp.bfloat16


def _dot(a, b):
    return jnp.dot(a, b, preferred_element_type=F32)


def _dot_nt(a, b):
    return lax.dot_general(a, b, (((1,), (1,)), ((), ())), preferred_element_type=F32)


def _layernorm(x):
    m = jnp.mean(x, axis=-1, keepdims=True)
    d = x - m
    v = jnp.mean(d * d, axis=-1, keepdims=True)
    return d * lax.rsqrt(v + EPS)


def _gelu(x):
    c = math.sqrt(2.0 / math.pi)
    return (0.5 * x) * (1.0 + jnp.tanh(x * (c + (c * 0.044715) * (x * x))))


def _kernel(x_hbm, wqkv_hbm, wo_hbm, wg_hbm, wu_hbm, wd_hbm, c_ref, wmod_hbm, out_hbm,
            x_v, wqkv_v, wo_v, wgu_v, wd_v, wmod_v, wvt_v,
            k9, q9, vt, ot, s0, s1, qm0, qm1, x1_v, h2_v, out_v, sems, osems):
    nb1 = S // RB1
    cp_mod_a = pltpu.make_async_copy(wmod_hbm.at[:, pl.ds(0, 2 * D)], wmod_v.at[:, pl.ds(0, 2 * D)], sems.at[0])
    cp_mod_b = pltpu.make_async_copy(wmod_hbm.at[:, pl.ds(2 * D, 4 * D)], wmod_v.at[:, pl.ds(2 * D, 4 * D)], sems.at[1])
    cp_wqkv = pltpu.make_async_copy(wqkv_hbm, wqkv_v, sems.at[2])
    cp_wo = pltpu.make_async_copy(wo_hbm, wo_v, sems.at[3])
    nt = F - FMAIN
    cp_wg = pltpu.make_async_copy(wg_hbm.at[pl.ds(0, FMAIN)], wgu_v.at[pl.ds(0, FMAIN)], sems.at[4])
    cp_wu = pltpu.make_async_copy(wu_hbm.at[pl.ds(0, FMAIN)], wgu_v.at[pl.ds(FMAIN, FMAIN)], sems.at[5])
    cp_wg2 = pltpu.make_async_copy(wg_hbm.at[pl.ds(FMAIN, nt)], wgu_v.at[pl.ds(2 * FMAIN, nt)], sems.at[7])
    cp_wu2 = pltpu.make_async_copy(wu_hbm.at[pl.ds(FMAIN, nt)], wgu_v.at[pl.ds(2 * FMAIN + nt, nt)], sems.at[8])
    cp_wd = pltpu.make_async_copy(wd_hbm, wd_v, sems.at[6])
    cp_x = [pltpu.make_async_copy(x_hbm.at[pl.ds(b * RB1, RB1)], x_v.at[pl.ds(b * RB1, RB1)], sems.at[9 + b])
            for b in range(nb1)]
    cp_mod_a.start()
    cp_x[0].start()
    cp_wqkv.start()
    for b in range(1, nb1):
        cp_x[b].start()

    cf = c_ref[...].astype(F32)
    sc = jnp.broadcast_to(cf * jax.nn.sigmoid(cf), (16, D)).astype(BF16)
    cp_mod_a.wait()
    mod_a = _dot(sc, wmod_v[:, 0:2 * D])[0:1]
    sa = mod_a[:, 0:D]
    ca1 = 1.0 + mod_a[:, D:2 * D]

    cp_x[0].wait()
    cp_wqkv.wait()
    for cp in (cp_mod_b, cp_wo, cp_wg, cp_wu, cp_wg2, cp_wu2, cp_wd):
        cp.start()
    for b in range(1, nb1):
        cp_x[b].wait()
    wvt_v[...] = wqkv_v[:, 2 * D:3 * D].T

    def qkv_block(b, carry):
        r0 = pl.multiple_of(b * RB1, RB1)
        rows = pl.ds(r0, RB1)
        h = (_layernorm(x_v[rows, :].astype(F32)) * ca1 + sa).astype(BF16)
        upper = lax.broadcasted_iota(jnp.int32, (RB1, LANES), 1) >= 64

        def put(dst, val):
            for t in range(NT):
                vt_ = val[:, t * LANES:(t + 1) * LANES]
                dst[t, rows, :] = vt_.astype(BF16)
                if t + 1 < NT:
                    dst[NT + t, rows, :] = jnp.where(upper, vt_, val[:, (t + 1) * LANES:(t + 2) * LANES]).astype(BF16)

        put(k9, _dot(h, wqkv_v[:, D:2 * D]))
        put(q9, _dot(h, wqkv_v[:, 0:D]) * QSCALE)
        vt[:, rows] = _dot_nt(wvt_v[...], h).astype(BF16).astype(F32)
        return carry

    lax.fori_loop(0, nb1, qkv_block, 0)

    def head_info(item):
        hd = item & (H - 1)
        q0 = pl.multiple_of(((item >> 5) & (S // QB - 1)) * QB, QB)
        lo = hd * DH
        t = lo >> 7
        off = lo & (LANES - 1)
        straddle = (off + DH > LANES).astype(jnp.int32)
        return t + NT * straddle, t, t + straddle, off, q0

    def build_q(item, qm):
        kt, t_hi, t_lo, off, q0 = head_info(item)
        lane = lax.broadcasted_iota(jnp.int32, (QB // 2, LANES), 1)
        keep = ((lane + (LANES - off)) & (LANES - 1)) < DH
        bits = jnp.where(keep, pltpu.bitcast(q9[kt, pl.ds(q0, QB), :], jnp.int32), 0)
        qm[...] = pltpu.bitcast(bits, BF16)
        return kt

    def qk(kt, qm, s_w, c, m):
        s = _dot_nt(k9[kt, pl.ds(c * KC, KC), :], qm[...])
        s_w[pl.ds(c * KC, KC), :] = s
        cm = jnp.max(s.reshape(KC // 8, 8, QB), axis=0)
        return cm if m is None else jnp.maximum(m, cm)

    sub = lax.broadcasted_iota(jnp.int32, (8, KC), 0)

    def pv(vrow, odd, s_r, c, m, acc):
        p = jnp.exp2(s_r[pl.ds(c * KC, KC), :] - m)
        cols = pl.ds(c * KC, KC)
        if not odd:
            v = jnp.concatenate([vt[pl.ds(vrow, 16), cols],
                                 jnp.where(sub < 4, vt[pl.ds(pl.multiple_of(vrow + 16, 8), 8), cols], 1.0)], axis=0)
        else:
            v = jnp.concatenate([jnp.where(sub >= 4, vt[pl.ds(pl.multiple_of(vrow + 16, 8), 8), cols], 1.0),
                                 vt[pl.ds(pl.multiple_of(vrow + 24, 8), 16), cols]], axis=0)
        o = _dot(v, p)
        return o if acc is None else acc + o

    def finish_max(m):
        return jnp.max(m, axis=0, keepdims=True)

    kt0 = build_q(jnp.int32(0), qm0)
    kt1 = build_q(jnp.int32(1), qm1)
    m = None
    for c in range(NCH):
        m = qk(kt0, qm0, s0, c, m)
    m_even = finish_max(m)
    m = None
    for c in range(SKEW):
        m = qk(kt1, qm1, s1, c, m)

    def pair(i, carry):
        m_even, m_part = carry
        item = 2 * i
        kt_a = head_info(item + 1)[0]
        q0 = head_info(item)[4]
        vrow = pl.multiple_of((i & (H // 2 - 1)) * (2 * DH), 8)
        kt_b = build_q(item + 2, qm0)
        acc_a = None
        for c in range(NCH):
            if c + SKEW < NCH:
                m_part = qk(kt_a, qm1, s1, c + SKEW, m_part)
                if c + SKEW == NCH - 1:
                    m_odd = finish_max(m_part)
                    m_part = None
            else:
                m_part = qk(kt_b, qm0, s0, c + SKEW - NCH, m_part)
            acc_a = pv(vrow, False, s0, c, m_even, acc_a)
        kt_c = build_q(item + 3, qm1)
        acc_b = None
        for c in range(NCH):
            last = c == NCH - 1
            if last:
                acc_b = pv(vrow, True, s1, c, m_odd, acc_b)
            if c + SKEW < NCH:
                m_part = qk(kt_b, qm0, s0, c + SKEW, m_part)
                if c + SKEW == NCH - 1:
                    m_even = finish_max(m_part)
                    m_part = None
            else:
                m_part = qk(kt_c, qm1, s1, c + SKEW - NCH, m_part)
            if not last:
                acc_b = pv(vrow, True, s1, c, m_odd, acc_b)
        ra = 1.0 / acc_a[20:21]
        rb = 1.0 / acc_b[0:1]
        cols = pl.ds(q0, QB)
        sub_q = lax.broadcasted_iota(jnp.int32, (8, QB), 0)
        ot[pl.ds(vrow, 16), cols] = acc_a[0:16] * ra
        ot[pl.ds(pl.multiple_of(vrow + 16, 8), 8), cols] = jnp.where(sub_q < 4, acc_a[16:24] * ra, acc_b[0:8] * rb)
        ot[pl.ds(pl.multiple_of(vrow + 24, 8), 16), cols] = acc_b[8:24] * rb
        return m_even, m_part

    lax.fori_loop(0, (S // QB) * (H // 2), pair, (m_even, m))

    for cp in (cp_mod_b, cp_wo, cp_wg, cp_wu, cp_wg2, cp_wu2, cp_wd):
        cp.wait()
    mod_b = _dot(sc, wmod_v[:, 2 * D:6 * D])[0:1]
    ga = mod_b[:, 0:D]
    sb = mod_b[:, D:2 * D]
    cb1 = 1.0 + mod_b[:, 2 * D:3 * D]
    gb = mod_b[:, 3 * D:4 * D]

    def proj_block(b, carry):
        r0 = pl.multiple_of(b * RB1, RB1)
        rows = pl.ds(r0, RB1)
        o = ot[:, rows].T.astype(BF16)
        x1 = x_v[rows, :].astype(F32) + ga * _dot(o, wo_v[...])
        x1_v[rows, :] = x1
        h2_v[rows, :] = (_layernorm(x1) * cb1 + sb).astype(BF16)
        return carry

    lax.fori_loop(0, nb1, proj_block, 0)

    def out_copy(b):
        rows = pl.ds(pl.multiple_of(b * RB3, RB3), RB3)
        return pltpu.make_async_copy(out_v.at[rows], out_hbm.at[rows], osems.at[b])

    def ffn_block(b, carry):
        r0 = pl.multiple_of(b * RB3, RB3)
        rows = pl.ds(r0, RB3)
        h2 = h2_v[rows, :]
        g = _dot_nt(h2, wgu_v[0:FMAIN, :])
        u = _dot_nt(h2, wgu_v[FMAIN:2 * FMAIN, :])
        gu = _dot_nt(h2, wgu_v[2 * FMAIN:2 * F, :])
        a = (_gelu(g) * u).astype(BF16)
        a_tail = (_gelu(gu) * pltpu.roll(gu, 64, 1))[:, 0:F - FMAIN].astype(BF16)
        y = _dot(a, wd_v[0:FMAIN, :]) + _dot(a_tail, wd_v[FMAIN:F, :])
        out_v[rows, :] = (x1_v[rows, :] + gb * y).astype(out_v.dtype)
        out_copy(b).start()
        return carry

    lax.fori_loop(0, S // RB3, ffn_block, 0)
    for b in range(S // RB3):
        out_copy(b).wait()


@jax.jit
def pallas_adaLN_cond__mha_block__geglu_ffn__prompt_kernel(
    A_x, A_wqkv, A_wo, B_x, B_w_gate, B_w_up, B_w_down, c, w_mod,
):
    del B_x
    any_spec = pl.BlockSpec(memory_space=pltpu.HBM)
    out = pl.pallas_call(
        _kernel,
        out_shape=jax.ShapeDtypeStruct((S, D), A_x.dtype),
        in_specs=[any_spec] * 6 + [pl.BlockSpec(memory_space=pltpu.VMEM), any_spec],
        out_specs=any_spec,
        scratch_shapes=[
            pltpu.VMEM((S, D), BF16),
            pltpu.VMEM((D, 3 * D), BF16),
            pltpu.VMEM((D, D), BF16),
            pltpu.VMEM((2 * F, D), BF16),
            pltpu.VMEM((F, D), BF16),
            pltpu.VMEM((D, 6 * D), BF16),
            pltpu.VMEM((D, D), BF16),
            pltpu.VMEM((2 * NT - 1, S, LANES), BF16),
            pltpu.VMEM((2 * NT - 1, S, LANES), BF16),
            pltpu.VMEM((D, S), F32),
            pltpu.VMEM((D, S), F32),
            pltpu.VMEM((S, QB), F32),
            pltpu.VMEM((S, QB), F32),
            pltpu.VMEM((QB, LANES), BF16),
            pltpu.VMEM((QB, LANES), BF16),
            pltpu.VMEM((S, D), F32),
            pltpu.VMEM((S, D), BF16),
            pltpu.VMEM((S, D), A_x.dtype),
            pltpu.SemaphoreType.DMA((9 + S // RB1,)),
            pltpu.SemaphoreType.DMA((S // RB3,)),
        ],
        compiler_params=pltpu.CompilerParams(vmem_limit_bytes=110 * 1024 * 1024),
        name="adaln_block",
    )(A_x.reshape(S, D), A_wqkv, A_wo, B_w_gate.T, B_w_up.T, B_w_down, c, w_mod)
    return out.reshape(1, S, D)
```

```python
import functools
import math

import jax
import jax.numpy as jnp
from jax import lax
import jax.experimental.pallas as pl
import jax.experimental.pallas.tpu as pltpu

F32, BF16, I32 = jnp.float32, jnp.bfloat16, jnp.int32

S, D, H, DH, F = 2048, 640, 32, 20, 1728
EPS = 1e-5
LANES = 128
NT = D // LANES
HALF = D // 2
DM = 512
FM, FP = 1536, 1792
QB = 512
NQ = S // QB
QTILES = QB // LANES

KC = 128
NCH = S // KC
HC = NCH // 2
RV = 16
RM = KC - RV
PIECES = RM // 16
STEPS = NQ * NCH
HEADS_PER_TRIP = 2
RING = 4
LAG = 2
KB0 = NQ * DH
KB1 = KB0 + NCH * DH // 2
P_LOADS = (1, 3, 4, 4, 4, 0, 0)
DIMS = (4, 3, 3, 3, 3, 3, 1)
DIMS_LAST = (6, 4, 4, 3, 3, 0, 0)
Q_FILLS = (0, 1, 2)
K_FILLS = (1, 2, 3, 5, 6)

UP_ROWS = 576
OUT_TAIL = 128

QSCALE = DH ** -0.5 * math.log2(math.e)
SUM_LO, ACC_HI = 2.0 ** -60, 2.0 ** 100
GELU_IN = (math.sqrt(2.0 / math.pi) * 0.044715) ** (1.0 / 3.0)

_PRODUCTS = {
    1: (((1, 0, 0), (1, 1, 1)), ((1, 0, 0), (1, 1, 1))),
    2: (((1, 1, 0), (1, 1, 1)), ((1, 0, 0),)),
    3: (((1, 0, 0),), ((1, 0, 1), (-1, 1, 1))),
    4: (((1, 1, 1),), ((1, 1, 0), (-1, 0, 0))),
    5: (((1, 0, 0), (1, 0, 1)), ((1, 1, 1),)),
    6: (((1, 1, 0), (-1, 0, 0)), ((1, 0, 0), (1, 0, 1))),
    7: (((1, 0, 1), (-1, 1, 1)), ((1, 1, 0), (1, 1, 1))),
}
_OUTPUTS = {
    (0, 0): ((1, 1), (1, 4), (-1, 5), (1, 7)),
    (0, 1): ((1, 3), (1, 5)),
    (1, 0): ((1, 2), (1, 4)),
    (1, 1): ((1, 1), (-1, 2), (1, 3), (1, 6)),
}
ORDER_QKV = ((5, 1, 2, 3, 4, 7, 6),)
ORDER_PROJ = ((2, 5, 4, 1, 7, 3, 6),)
ORDER_UP1 = ((2, 5, 1, 4, 7, 3, 6),)
ORDER_UP2 = ((3, 5, 1, 7, 2, 6, 4), (5, 1, 2, 3, 4, 7, 6))
ORDER_TAIL = ((2, 4, 1, 5, 7, 3, 6),)
ORDER_DOWN = ((4, 3, 2, 1, 5, 7, 6), (5, 1, 2, 3, 4, 7, 6))


def _signed_sum(terms):
    terms = sorted(terms, key=lambda t: -t[0])
    out = terms[0][1]
    for sign, val in terms[1:]:
        out = out + val if sign > 0 else out - val
    return out


def _strassen(a, b, orders, multiply, emit):
    if not orders:
        emit(0, 0, multiply(lambda: a(0, 0), lambda: b(0, 0)))
        return
    n = 1 << (len(orders) - 1)
    done = {}

    def operand(get, terms):
        @functools.cache
        def block(i, j):
            vals = [(s, get(x * n + i, y * n + j)) for s, x, y in terms]
            return vals[0][1] if len(vals) == 1 else _signed_sum([(s, v.astype(F32)) for s, v in vals])
        return block

    def collect(p, i, j, val):
        done[p, i, j] = val
        for (x, y), terms in _OUTPUTS.items():
            signs = [s for s, q in terms if q == p]
            if signs and all((q, i, j) in done for _, q in terms):
                older = _signed_sum([(s, done[q, i, j]) for s, q in terms if q != p])
                emit(x * n + i, y * n + j, val + older if signs[0] > 0 else older - val)

    for p in orders[0]:
        _strassen(operand(a, _PRODUCTS[p][0]), operand(b, _PRODUCTS[p][1]), orders[1:], multiply,
                  functools.partial(collect, p))


def _dot(a, b):
    return lax.dot_general(a, b, (((1,), (0,)), ((), ())), preferred_element_type=F32)


def _dot_nt(a, b):
    return lax.dot_general(a, b, (((1,), (1,)), ((), ())), preferred_element_type=F32)


def _normalize_lanes(x):
    d = x - jnp.mean(x, axis=1, keepdims=True)
    return d * lax.rsqrt(jnp.mean(d * d, axis=1, keepdims=True) + EPS)


def _mean_rows(x):
    parts = [x[r:r + 8] for r in range(0, x.shape[0], 8)]
    sums = [functools.reduce(lambda a, b: a + b, parts[k::4]) for k in range(4)]
    return jnp.sum((sums[0] + sums[1]) + (sums[2] + sums[3]), axis=0, keepdims=True) * (1.0 / x.shape[0])


def _gelu_scaled(y):
    return y * (1.0 + jnp.tanh(y * (math.sqrt(2.0 / math.pi) / GELU_IN + y * y)))


def _tile_lanes(v, n):
    return jnp.concatenate([v] * (n // LANES), axis=1)


def _key_tile(hd):
    lo = hd * DH
    off = lo & (LANES - 1)
    return (lo >> 7) + NT * (off + DH > LANES).astype(I32), off


def _aligned_keys(tile, off):
    lane = lax.broadcasted_iota(I32, tile.shape, 1)
    return jnp.take_along_axis(tile, (lane + off) & (LANES - 1), axis=1)


def _kernel(x_hbm, wqkv_hbm, wo_hbm, wg_hbm, wu_hbm, wd_hbm, c_hbm, wmod_hbm, out_hbm,
            c_v, x_v, wo_v, wg_v, wu_v, wd_v, wmod_v, wot, wdt, xt, ot, mod_v, zero_s, sems):
    @pl.loop(0, 2)
    def _(i):
        zero_s[i] = 0

    def pin(buf, row, val):
        buf[pl.ds(pl.multiple_of(zero_s[0] + row, val.shape[0]), val.shape[0]), 0:LANES] = val

    copies = []

    def copy(src, dst):
        copies.append(pltpu.make_async_copy(src, dst, sems.at[len(copies)]))
        return copies[-1]

    def mod_copy(lo, n):
        return copy(wmod_hbm.at[:, pl.ds(lo, n)], wmod_v.at[:, pl.ds(lo, n)])

    def mod(lo, n):
        cf = c_v[0].astype(F32)
        return _dot(jnp.broadcast_to(cf * jax.nn.sigmoid(cf), (8, D)), wmod_v[:, lo:lo + n])[0:1]

    def transpose(src, dst):
        def job(lo, n):
            dst[:, pl.ds(pl.multiple_of(zero_s[0] + lo, LANES), n)] = src[pl.ds(pl.multiple_of(lo, LANES), n), :].T
        return job

    late = [copy(wo_hbm, wo_v), copy(wd_hbm, wd_v.at[pl.ds(0, F)]), mod_copy(2 * D, 4 * D),
            copy(wg_hbm, wg_v), copy(wu_hbm, wu_v)]

    def attention_half(kv, km, kh, qt, vt, bc, ring, part):
        def key_slot(c, d):
            return KB0 + (c * DH + d) // 2, slice(None), pl.ds(d % 2 * 2 * LANES, 2 * LANES)

        def fill_head_keys(where, lo, n):
            t, off = where
            kh[pl.ds(8 * lo, 8 * n), :] = _aligned_keys(km[t, pl.ds(8 * lo, 8 * n), :], off)

        def broadcast_keys(where, c, dims):
            t, off = where
            keys = kv[t, pl.ds(c * RV, RV), :]
            for d in dims:
                val = jnp.take_along_axis(keys, jnp.full((RV, LANES), (off + d) & (LANES - 1), I32), axis=1)
                bc[key_slot(c, d)] = jnp.concatenate([val[0:8], val[8:16]], axis=1)

        def broadcast_queries(hd, blk, dims):
            for d in dims:
                rows = qt[hd, pl.ds(d // 8 * 8, 8), pl.ds(blk * QB, QB)]
                bc[blk * DH + d] = jnp.broadcast_to(rows[d % 8:d % 8 + 1], (8, QB))

        def project(wqkv_v, wt_tail, h_v, acc_v, kt, *wt):
            blocks = [pl.ds(b * QB, QB) for b in range(NQ)]
            cp_x = [copy(x_hbm.at[rows], x_v.at[rows]) for rows in blocks]
            cp_tail = [copy(c_hbm, c_v.at[0]), mod_copy(DM, D - DM), mod_copy(D + DM, D - DM),
                       copy(wqkv_hbm.at[pl.ds(DM, D - DM)], wqkv_v.at[pl.ds(DM, D - DM)])]
            cp_mod = [mod_copy(0, DM), mod_copy(D, DM)]
            w_parts = [(pl.ds(0, DM), pl.ds(kind * D, D)) for kind in (1, 0, 2)]
            cp_w = [copy(wqkv_hbm.at[part_], wqkv_v.at[part_]) for part_ in w_parts]
            for cp in cp_x[:1] + cp_tail + cp_x[1:] + cp_mod + cp_w:
                cp.start()

            def normalize(lo, n):
                h_v[pl.ds(lo, n), :] = _normalize_lanes(x_v[pl.ds(lo, n), :].astype(F32))

            def tail_pass(b, lo, hi, normalize_next):
                val = _dot_nt(wt_tail[lo:hi, :], h_v[blocks[b], DM:D] * ca1_tail + sa_tail)
                if normalize_next:
                    for k in range(16):
                        r = (hi - lo) // 8 * k // 18 * 8
                        pin(x_v, S, pltpu.bitcast(val[r:r + 8, 0:LANES], BF16))
                        normalize((b + 1) * QB + k * QB // 16, QB // 16)
                acc_v[lo:hi, blocks[b]] = val

            cp_x[0].wait()
            normalize(0, QB)
            for cp in cp_tail:
                cp.wait()
            sa_tail, ca1_tail = mod(DM, D - DM), 1.0 + mod(D + DM, D - DM)
            transpose(wqkv_v.at[pl.ds(DM, D - DM)], wt_tail)(0, D - DM)
            tail_pass(0, 0, D, False)
            for b in range(NQ - 1):
                cp_x[b + 1].wait()
                tail_pass(b, 0 if b else D, 3 * D, True)
            for cp in cp_mod:
                cp.wait()
            sa, ca1 = mod(0, DM), 1.0 + mod(D, DM)
            tail_pass(NQ - 1, 0, 3 * D, False)

            def transpose_w(kind, lo, n):
                wt[kind][:, pl.ds(pl.multiple_of(zero_s[0] + lo, LANES), n)] = (
                    wqkv_v[pl.ds(lo, n), pl.ds(kind * D, D)].T)

            def split_keys(c):
                tiles = [kt[pl.ds(t * LANES, LANES), pl.ds(c * KC, KC)].T for t in range(NT)]
                upper = lax.broadcasted_iota(I32, (KC, LANES), 1) >= LANES // 2
                tiles += [jnp.where(upper, tiles[t], tiles[t + 1]) for t in range(NT - 1)]
                for t, keys in enumerate(tiles):
                    kv[t, pl.ds(c * RV, RV), :] = keys[0:RV]
                    km[t, pl.ds(c * RM // 2, RM // 2), :] = pltpu.bitcast(keys[RV:KC].astype(BF16), I32)

            def first_keys(c):
                fill_head_keys(_key_tile(jnp.int32(0)), c * PIECES, PIECES)
                broadcast_keys(_key_tile(jnp.int32(0)), c, range(DH))

            def store_qkv(kind, i, cols, val):
                val = val + acc_v[pl.ds(kind * D + i * HALF, HALF), cols]
                if kind == 1:
                    kt[pl.ds(i * HALF, HALF), cols] = val
                    return
                low = lax.broadcasted_iota(I32, (8, QB), 0) < 4
                for u in range(0, HALF, 2 * DH):
                    v = [val[u + r:u + r + 8] for r in range(0, 2 * DH, 8)]
                    hd = (i * HALF + u) // DH
                    if kind == 0:
                        v = [r * QSCALE for r in v]
                        w = [pltpu.roll(r, 4, 0) for r in v[2:]]
                        qt[hd, :, cols] = jnp.concatenate([v[0], v[1], jnp.where(low, v[2], 0.0)], axis=0)
                        qt[hd + 1, :, cols] = jnp.concatenate(
                            [jnp.where(low, w[0], w[1]), jnp.where(low, w[1], w[2]), jnp.where(low, w[2], 0.0)], axis=0)
                    else:
                        vt[hd, :, cols] = jnp.concatenate([v[0], v[1], jnp.where(low, v[2], 1.0)], axis=0)
                        vt[hd + 1, :, cols] = jnp.concatenate([jnp.where(low, 1.0, v[2]), v[3], v[4]], axis=0)

            previous = []

            def main_pass(kind, b, jobs):
                left = [7]

                def multiply(lhs, rhs):
                    for _ in range(pl.cdiv(len(jobs), left[0])):
                        pin(kt, D, previous[0][0:8, 0:LANES])
                        jobs.pop(0)()
                    left[0] -= 1
                    previous[:] = [_dot_nt(lhs(), rhs())]
                    return previous[0]

                def h_block(k, t):
                    lanes = slice(k * DM // 2, (k + 1) * DM // 2)
                    return h_v[blocks[b + t], lanes] * ca1[:, lanes] + sa[:, lanes]

                _strassen(lambda i, k: wt[kind][pl.ds(i * HALF, HALF), pl.ds(k * DM // 2, DM // 2)], h_block,
                          ORDER_QKV, multiply, lambda i, t, val: store_qkv(kind, i, blocks[b + t], val))

            job = functools.partial
            cp_w[0].wait()
            transpose_w(1, 0, DM)
            main_pass(1, 0, [])
            cp_w[1].wait()
            cp_w[2].wait()
            for cp in late:
                cp.start()
            main_pass(1, 2, [job(transpose_w, kind, lo, LANES) for kind in (0, 2) for lo in range(0, DM, LANES)])
            main_pass(0, 0, [job(transpose(x_v, xt), lo, LANES) for lo in range(0, S, LANES)])
            main_pass(0, 2, [job(split_keys, c) for c in range(HC)])
            main_pass(2, 0, [job(first_keys, c) for c in range(HC)]
                      + [job(broadcast_queries, 0, b, range(DH)) for b in range(NQ - 1)])
            main_pass(2, 2, [job(split_keys, c) for c in range(HC, NCH)])

        pl.run_scoped(project, pltpu.VMEM((D, 3 * D), BF16), pltpu.VMEM((3 * D, D - DM), BF16),
                      pltpu.VMEM((S, D), F32), pltpu.VMEM((3 * D, S), F32), pltpu.VMEM((D + 8, S), F32),
                      *[pltpu.VMEM((D, DM), BF16)] * 3)

        def step(n):
            half, rest = divmod(n % STEPS, NQ * HC)
            blk, c = divmod(rest, HC)
            return blk, half * HC + c

        def load_p(n, lo, rows):
            return ring[n % RING, pl.ds(8 * lo, 8 * rows), :]

        def accumulate(hd, blk, c, p, acc):
            o = _dot(vt[hd, :, pl.ds(c * KC, KC)], p)
            if c == HC:
                acc = part[zero_s[0] + blk]
            acc = o if c == 0 else o + acc
            if c % HC == HC - 1:
                part[blk] = acc
            return acc

        def store_output(hd, cols, acc):
            odd = hd & 1
            sub = lax.broadcasted_iota(I32, (8, LANES), 0)
            total = jnp.where(odd == 1, acc[0:1], acc[23:24])
            o = acc * (1.0 / total)
            r = pl.multiple_of(((hd * DH) >> 3) << 3, 8)
            ot[pl.ds(r, 8), cols] = jnp.where(sub < 4 * odd, ot[pl.ds(r, 8), cols], o[0:8])
            ot[pl.ds(pl.multiple_of(r + 8, 8), 16), cols] = o[8:24]
            return total

        def finish(hd, blk, u, unsafe):
            acc = part[zero_s[0] + blk, :, pl.ds(u * LANES, LANES)]
            total = store_output(hd, pl.ds(blk * QB + u * LANES, LANES), acc)
            mag = jnp.abs(acc)
            ok = (mag[0:8] < ACC_HI) & (mag[8:16] < ACC_HI) & (mag[16:24] < ACC_HI) & (total > SUM_LO)
            return jnp.where(ok, unsafe, 1.0)

        def head(hd, acc, unsafe, p, last):
            z = zero_s[0]
            prv, nxt = jnp.maximum(hd - 1, 0), jnp.minimum(hd + 1, H - 1)
            keys = (_key_tile(hd), _key_tile(nxt))
            for n in range(STEPS):
                blk, c = step(n)
                half, rest = divmod(n, NQ * HC)
                lhs = pltpu.bitcast(kh[pl.ds(c * RM // 2, RM // 2), :], BF16)[:, 0:24]
                pm = jnp.exp2(_dot(lhs, qt[hd, :, pl.ds(blk * QB, QB)]))
                p_next = []
                d, r = 0, KC // 8
                for j in range(PIECES):
                    ring[n % RING, pl.ds(RV + 16 * j, 16), :] = pm[16 * j:16 * j + 16]
                    token = pm[16 * j:16 * j + 8, 0:LANES]
                    ring[z + RING, 0:8, 0:LANES] = token
                    bc[z + KB1, :, 0:LANES] = token
                    if P_LOADS[j]:
                        r -= P_LOADS[j]
                        p_next.insert(0, load_p(n - LAG + 1, r, P_LOADS[j]))
                    for _ in range((DIMS_LAST if last and n + 1 == STEPS else DIMS)[j]):
                        kk, qq = bc[key_slot(c, d)], bc[blk * DH + d]
                        prod = jnp.concatenate(
                            [_tile_lanes(kk[:, 0:LANES], QB) * qq, _tile_lanes(kk[:, LANES:], QB) * qq], axis=0)
                        scores = prod if d == 0 else scores + prod
                        d += 1
                    dims = [e for e in range(3 * (c % HC), min(3 * (c % HC) + 3, DH)) if Q_FILLS[e % 3] == j]
                    if half and blk:
                        broadcast_queries(nxt, blk - 1, dims)
                    if not half and not blk:
                        broadcast_queries(hd, NQ - 1, dims)
                    if j in K_FILLS:
                        broadcast_keys(keys[half], (1 - half) * HC + rest // 4, [5 * (rest % 4) + K_FILLS.index(j)])
                    if j == 2 and rest < HC * PIECES // 4:
                        fill_head_keys(keys[half], (1 - half) * HC * PIECES + 4 * rest, 4)
                    if j == 0:
                        acc = accumulate(prv if n < LAG else hd, *step(n - LAG), p, acc)
                        after, u = step(n - LAG - 2)
                        if u % HC < QTILES and (after > 0) == (u >= HC):
                            part[z + NQ, 0:8, 0:LANES] = token
                            unsafe = finish(hd if after else prv, (after - 1) % NQ, u % HC, unsafe)
                ring[n % RING, 0:RV, :] = jnp.exp2(scores)
                p = jnp.concatenate(p_next, axis=0)
            return acc, unsafe, p

        def trip(i, carry):
            carry = (*carry, load_p(-LAG, 0, KC // 8))
            for k in range(HEADS_PER_TRIP):
                carry = head(HEADS_PER_TRIP * i + k, *carry, k + 1 == HEADS_PER_TRIP)
            return carry[:2]

        for n in range(-LAG, 0):
            ring[n % RING] = jnp.zeros((KC, QB), F32)
        acc, unsafe = lax.fori_loop(0, H // HEADS_PER_TRIP, trip,
                                    (jnp.ones((24, QB), F32), jnp.zeros((8, LANES), F32)))
        for cp in late:
            cp.wait()
        transpose(wo_v, wot)(0, D)
        mod_v[...] = jnp.broadcast_to(mod(2 * D, 4 * D), mod_v.shape)
        for n in range(-LAG, 0):
            acc = accumulate(jnp.int32(H - 1), *step(n), load_p(n, 0, KC // 8), acc)
        for u in range(QTILES):
            unsafe = finish(jnp.int32(H - 1), NQ - 1, u, unsafe)

        @pl.when(jnp.max(unsafe) > 0.0)
        def _():
            @pl.loop(0, H * S // LANES)
            def _(i):
                hd = i >> 4
                cols = pl.ds(pl.multiple_of((i & (S // LANES - 1)) * LANES, LANES), LANES)
                q = qt[hd, :, cols]
                t, off = _key_tile(hd)
                sm = _dot(pltpu.bitcast(_aligned_keys(km[t], off), BF16)[:, 0:24], q)
                sv = _dot(_aligned_keys(kv[t], off)[:, 0:24], q)
                top = jnp.maximum(jnp.max(sm, axis=0, keepdims=True), jnp.max(sv, axis=0, keepdims=True))
                pm, pv = jnp.exp2(sm - top), jnp.exp2(sv - top)
                p = [x for c in range(NCH) for x in (pv[c * RV:(c + 1) * RV], pm[c * RM:(c + 1) * RM])]
                store_output(hd, cols, _dot(vt[hd], jnp.concatenate(p, axis=0)))

    pl.run_scoped(
        attention_half,
        pltpu.VMEM((2 * NT - 1, NCH * RV, LANES), F32),
        pltpu.VMEM((2 * NT - 1, NCH * RM // 2, LANES), I32),
        pltpu.VMEM((NCH * RM // 2, LANES), I32),
        pltpu.VMEM((H, 24, S), F32),
        pltpu.VMEM((H, 24, S), F32),
        pltpu.VMEM((KB1 + 1, 8, QB), F32),
        pltpu.VMEM((RING + 1, KC, QB), F32),
        pltpu.VMEM((NQ + 1, 24, QB), F32),
    )

    def ffn_half(x1, h2, act, out_v):
        wd_v[F:FP, :] = jnp.zeros((FP - F, D), BF16)
        act[F:FP, :] = jnp.zeros((FP - F, S), F32)
        ga, sb, cb1, gb = (
            jnp.concatenate([(one + mod_v[:, k * D:(k + 1) * D]) * scale] * (LANES // 8), axis=0).T
            for k, (one, scale) in enumerate(((0.0, 1.0), (0.0, GELU_IN), (1.0, GELU_IN), (0.0, 0.5 / GELU_IN ** 2))))
        jobs = []

        def multiply(lhs, rhs, per_product=0):
            lhs, rhs = lhs(), rhs()
            for _ in range(min(per_product, len(jobs))):
                jobs.pop(0)()
            return _dot(lhs, rhs)

        def normalize(tile):
            cols = pl.ds(tile * LANES, LANES)
            stats = []

            def mean():
                stats.append(_mean_rows(x1[:, cols]))

            def scale():
                d = x1[:, cols] - stats[0]
                stats.append(lax.rsqrt(_mean_rows(d * d) + EPS))

            def apply(rows):
                h2[rows, cols] = (x1[rows, cols] - stats[0]) * stats[1] * cb1[rows] + sb[rows]

            return [mean, scale, functools.partial(apply, slice(0, HALF)), functools.partial(apply, slice(HALF, D))]

        for b in range(0, NQ, 2):
            seen = set()

            def residual(i, t, val):
                rows, cols = slice(i * HALF, (i + 1) * HALF), pl.ds((b + t) * QB, QB)
                val = _dot(wot[rows, DM:D], ot[DM:D, cols]) + val
                x1[rows, cols] = xt[rows, cols].astype(F32) + _tile_lanes(ga[rows], QB) * val
                if t in seen:
                    for u in range(QTILES):
                        jobs.extend(normalize((b + t) * QTILES + u))
                seen.add(t)

            _strassen(lambda i, k: wot[pl.ds(i * HALF, HALF), pl.ds(k * DM // 2, DM // 2)],
                      lambda k, t: ot[pl.ds(k * DM // 2, DM // 2), pl.ds((b + t) * QB, QB)],
                      ORDER_PROJ, functools.partial(multiply, per_product=4), residual)

        def gated(chunk, b, orders):
            n = 1 << len(orders)
            m = 2 * UP_ROWS // n
            other = {}

            def weights(i, lanes):
                rows = pl.ds(pl.multiple_of(chunk * UP_ROWS, 64) + i % (n // 2) * m, m)
                return rows, (wg_v if i < n // 2 else wu_v)[rows, lanes]

            def activate(i, t, val):
                cols = pl.ds((b + t) * QB, QB)
                rows, w = weights(i, slice(DM, D))
                val = _dot(w, h2[DM:D, cols]) + val
                if i < n // 2:
                    val = _gelu_scaled(val)
                if (i % (n // 2), t) in other:
                    act[rows, cols] = other[i % (n // 2), t] * val
                other[i % (n // 2), t] = val

            _strassen(lambda i, k: weights(i, pl.ds(k * DM // n, DM // n))[1],
                      lambda k, t: h2[pl.ds(k * DM // n, DM // n), pl.ds((b + t) * QB, QB)],
                      orders, functools.partial(multiply, per_product=8), activate)

        def transpose_wd(chunk):
            n = pl.cdiv(FP // LANES, F // UP_ROWS)
            transpose(wd_v, wdt)(jnp.minimum(chunk * n, FP // LANES - n) * LANES, n * LANES)

        gated(0, 0, ORDER_UP1)
        transpose_wd(0)
        gated(0, 2, ORDER_UP1)

        @pl.loop(1, F // UP_ROWS)
        def _(chunk):
            transpose_wd(chunk)
            gated(chunk, 0, ORDER_UP2)

        tail = {}
        _strassen(lambda i, k: wdt[pl.ds(i * HALF, HALF), pl.ds(FM + k * LANES, LANES)],
                  lambda k, t: act[pl.ds(FM + k * LANES, LANES), pl.ds(t * QB, QB)],
                  ORDER_TAIL, multiply, lambda i, t, val: tail.update({(i, t): val}))
        parts = [{} for _ in range(NQ)]
        writes, due = [], []

        def write(lo, y):
            cols = pl.ds(lo, y.shape[1])
            out_v[cols, :] = (x1[:, cols] + _tile_lanes(gb, y.shape[1]) * y).astype(out_v.dtype).T
            writes.append(copy(out_v.at[cols], out_hbm.at[cols]))
            writes[-1].start()

        def multiply_in_time(lhs, rhs):
            for entry in due:
                if entry[0] == 0:
                    rows = pl.ds(pl.multiple_of(zero_s[0] + entry[1], 16), 16)
                    pin(act, FP, pltpu.bitcast(out_v[rows, 0:LANES], F32))
                entry[0] -= 1
            return _dot(lhs(), rhs())

        def gather(i, t, val):
            if t < NQ // 2:
                val = val + tail[i // 2, t][i % 2 * D // 4:(i % 2 + 1) * D // 4]
            parts[t][i] = val
            if t < NQ // 2 and len(parts[t]) == 4:
                write(t * QB, jnp.concatenate([parts[t][k] for k in range(4)], axis=0))
                due.append([7, t * QB])

        _strassen(lambda i, k: wdt[pl.ds(i * D // 4, D // 4), pl.ds(k * FM // 4, FM // 4)],
                  lambda k, t: act[pl.ds(k * FM // 4, FM // 4), pl.ds(t * QB, QB)],
                  ORDER_DOWN, multiply_in_time, gather)
        for lo in range(S // 2, S, OUT_TAIL):
            y = jnp.concatenate([parts[lo // QB][k][:, lo % QB:lo % QB + OUT_TAIL] for k in range(4)], axis=0)
            write(lo, multiply_in_time(lambda: wdt[:, FM:FP], lambda: act[FM:FP, pl.ds(lo, OUT_TAIL)]) + y)
        for cp in writes:
            cp.wait()

    pl.run_scoped(ffn_half, pltpu.VMEM((D, S), F32), pltpu.VMEM((D, S), F32), pltpu.VMEM((FP + 8, S), F32),
                  pltpu.VMEM((S, D), out_hbm.dtype))


@jax.jit
def pallas_adaLN_cond__mha_block__geglu_ffn__prompt_kernel(
    A_x: jax.Array,
    A_wqkv: jax.Array,
    A_wo: jax.Array,
    B_x: jax.Array,
    B_w_gate: jax.Array,
    B_w_up: jax.Array,
    B_w_down: jax.Array,
    c: jax.Array,
    w_mod: jax.Array,
):
    del B_x
    hbm = pl.BlockSpec(memory_space=pltpu.HBM)
    out = pl.pallas_call(
        _kernel,
        out_shape=jax.ShapeDtypeStruct((S, D), A_x.dtype),
        in_specs=[hbm] * 8,
        out_specs=hbm,
        scratch_shapes=[
            pltpu.VMEM((32, 1, D), BF16),
            pltpu.VMEM((S + 64, D), BF16),
            pltpu.VMEM((D, D), BF16),
            pltpu.VMEM((F, D), BF16),
            pltpu.VMEM((F, D), BF16),
            pltpu.VMEM((FP, D), BF16),
            pltpu.VMEM((D, 6 * D), BF16),
            pltpu.VMEM((D, D), BF16),
            pltpu.VMEM((D, FP), BF16),
            pltpu.VMEM((D, S), BF16),
            pltpu.VMEM((D, S), F32),
            pltpu.VMEM((8, 4 * D), F32),
            pltpu.SMEM((2,), I32),
            pltpu.SemaphoreType.DMA((18 + NQ // 2 + S // 2 // OUT_TAIL,)),
        ],
        compiler_params=pltpu.CompilerParams(vmem_limit_bytes=126 * 1024 * 1024),
        name="adaln_block",
    )(A_x.reshape(S, D), A_wqkv, A_wo, B_w_gate.T, B_w_up.T, B_w_down, c, w_mod)
    return out.reshape(1, S, D)
```

```python
import functools
import math

import jax
import jax.numpy as jnp
from jax import lax
import jax.experimental.pallas as pl
import jax.experimental.pallas.tpu as pltpu

F32, BF16, I32 = jnp.float32, jnp.bfloat16, jnp.int32

S, D, H, DH, F = 2048, 640, 32, 20, 1728
EPS = 1e-5
LANES = 128
NT = D // LANES
HALF = D // 2
DM = 512
FM, FP = 1536, 1792
QB = 512
NQ = S // QB
QTILES = QB // LANES

KC = 128
NCH = S // KC
HC = NCH // 2
RV = 16
RM = KC - RV
PIECES = RM // 16
STEPS = NQ * NCH
HEADS_PER_TRIP = 2
RING = 4
LAG = 2
KB0 = NQ * DH
KB1 = KB0 + NCH * DH // 2
P_LOADS = (3, 2, 3, 4, 4, 0, 0)
DIMS = (4, 3, 3, 3, 3, 3, 1)
DIMS_LAST = (7, 4, 4, 1, 3, 1, 0)
Q_FILLS = (2, 4)
K_FILLS = (1, 2, 3, 5, 6)

UP_FIRST = 192
UP_CHUNKS = 2
OUT_TAIL = 128

QSCALE = DH ** -0.5 * math.log2(math.e)
SUM_LO, ACC_HI = 2.0 ** -60, 2.0 ** 100
GELU_IN = (math.sqrt(2.0 / math.pi) * 0.044715) ** (1.0 / 3.0)

_PRODUCTS = {
    1: (((1, 0, 0), (1, 1, 1)), ((1, 0, 0), (1, 1, 1))),
    2: (((1, 1, 0), (1, 1, 1)), ((1, 0, 0),)),
    3: (((1, 0, 0),), ((1, 0, 1), (-1, 1, 1))),
    4: (((1, 1, 1),), ((1, 1, 0), (-1, 0, 0))),
    5: (((1, 0, 0), (1, 0, 1)), ((1, 1, 1),)),
    6: (((1, 1, 0), (-1, 0, 0)), ((1, 0, 0), (1, 0, 1))),
    7: (((1, 0, 1), (-1, 1, 1)), ((1, 1, 0), (1, 1, 1))),
}
_OUTPUTS = {
    (0, 0): ((1, 1), (1, 4), (-1, 5), (1, 7)),
    (0, 1): ((1, 3), (1, 5)),
    (1, 0): ((1, 2), (1, 4)),
    (1, 1): ((1, 1), (-1, 2), (1, 3), (1, 6)),
}
ORDER_QKV = ((2, 5, 4, 3, 1, 7, 6),)
ORDER_PROJ = ((5, 2, 4, 1, 7, 3, 6),)
ORDER_UP1 = ((2, 5, 1, 4, 7, 3, 6),)
ORDER_UP2 = ((2, 5, 3, 1, 4, 6, 7), (5, 2, 1, 4, 7, 3, 6))
ORDER_TAIL = ((2, 5, 1, 3, 4, 6, 7),)
ORDER_DOWN = ((2, 3, 1, 4, 5, 7, 6), (5, 1, 3, 2, 4, 6, 7))


def _signed_sum(terms):
    terms = sorted(terms, key=lambda t: -t[0])
    out = terms[0][1]
    for sign, val in terms[1:]:
        out = out + val if sign > 0 else out - val
    return out


def _strassen(a, b, orders, multiply, emit):
    if not orders:
        emit(0, 0, multiply(lambda: a(0, 0), lambda: b(0, 0)))
        return
    n = 1 << (len(orders) - 1)
    done = {}

    def operand(get, terms):
        @functools.cache
        def block(i, j):
            vals = [(s, get(x * n + i, y * n + j)) for s, x, y in terms]
            return vals[0][1] if len(vals) == 1 else _signed_sum([(s, v.astype(F32)) for s, v in vals])
        return block

    def collect(p, i, j, val):
        done[p, i, j] = val
        for (x, y), terms in _OUTPUTS.items():
            signs = [s for s, q in terms if q == p]
            if signs and all((q, i, j) in done for _, q in terms):
                older = _signed_sum([(s, done[q, i, j]) for s, q in terms if q != p])
                emit(x * n + i, y * n + j, val + older if signs[0] > 0 else older - val)

    for p in orders[0]:
        _strassen(operand(a, _PRODUCTS[p][0]), operand(b, _PRODUCTS[p][1]), orders[1:], multiply,
                  functools.partial(collect, p))


def _dot(a, b):
    return lax.dot_general(a, b, (((1,), (0,)), ((), ())), preferred_element_type=F32)


def _dot_nt(a, b):
    return lax.dot_general(a, b, (((1,), (1,)), ((), ())), preferred_element_type=F32)


def _normalize_lanes(x):
    d = x - jnp.mean(x, axis=1, keepdims=True)
    return d * lax.rsqrt(jnp.mean(d * d, axis=1, keepdims=True) + EPS)


def _mean_rows(x):
    parts = [x[r:r + 8] for r in range(0, x.shape[0], 8)]
    sums = [functools.reduce(lambda a, b: a + b, parts[k::4]) for k in range(4)]
    return jnp.sum((sums[0] + sums[1]) + (sums[2] + sums[3]), axis=0, keepdims=True) * (1.0 / x.shape[0])


def _gelu_scaled(y):
    return y * (1.0 + jnp.tanh(y * (math.sqrt(2.0 / math.pi) / GELU_IN + y * y)))


def _tile_lanes(v, n):
    return jnp.concatenate([v] * (n // LANES), axis=1)


def _key_tile(hd):
    lo = hd * DH
    off = lo & (LANES - 1)
    return (lo >> 7) + NT * (off + DH > LANES).astype(I32), off


def _aligned_keys(tile, off):
    lane = lax.broadcasted_iota(I32, tile.shape, 1)
    return jnp.take_along_axis(tile, (lane + off) & (LANES - 1), axis=1)


def _kernel(x_hbm, wqkv_hbm, wo_hbm, wg_hbm, wu_hbm, wd_hbm, c_hbm, wmod_hbm, out_hbm,
            c_v, x_v, wo_v, wg_v, wu_v, wd_v, wmod_v, wot, wdt, xt, ot, mod_v, zero_s, sems):
    @pl.loop(0, 2)
    def _(i):
        zero_s[i] = 0

    def pin(buf, row, val):
        buf[pl.ds(pl.multiple_of(zero_s[0] + row, val.shape[0]), val.shape[0]), 0:LANES] = val

    copies = []

    def copy(src, dst):
        copies.append(pltpu.make_async_copy(src, dst, sems.at[len(copies)]))
        return copies[-1]

    def mod_copy(lo, n):
        return copy(wmod_hbm.at[:, pl.ds(lo, n)], wmod_v.at[:, pl.ds(lo, n)])

    def mod(lo, n):
        cf = c_v[0].astype(F32)
        return _dot(jnp.broadcast_to(cf * jax.nn.sigmoid(cf), (8, D)), wmod_v[:, lo:lo + n])[0:1]

    def transpose(src, dst):
        def job(lo, n):
            dst[:, pl.ds(pl.multiple_of(zero_s[0] + lo, LANES), n)] = src[pl.ds(pl.multiple_of(lo, LANES), n), :].T
        return job

    late = [copy(wo_hbm, wo_v), copy(wd_hbm, wd_v.at[pl.ds(0, F)]), mod_copy(2 * D, 4 * D),
            copy(wg_hbm, wg_v), copy(wu_hbm, wu_v)]

    def attention_half(kv, km, kh, qt, vt, bc, ring, part, sums):
        def key_slot(c, d):
            return KB0 + (c * DH + d) // 2, slice(None), pl.ds(d % 2 * 2 * LANES, 2 * LANES)

        def fill_head_keys(where, lo, n):
            t, off = where
            kh[pl.ds(8 * lo, 8 * n), :] = _aligned_keys(km[t, pl.ds(8 * lo, 8 * n), :], off)

        def broadcast_keys(where, c, dims):
            t, off = where
            keys = kv[t, pl.ds(c * RV, RV), :]
            for d in dims:
                val = jnp.take_along_axis(keys, jnp.full((RV, LANES), (off + d) & (LANES - 1), I32), axis=1)
                bc[key_slot(c, d)] = jnp.concatenate([val[0:8], val[8:16]], axis=1)

        def broadcast_queries(hd, blk, dims):
            for d in dims:
                rows = qt[hd, pl.ds(d // 8 * 8, 8), pl.ds(blk * QB, QB)]
                bc[blk * DH + d] = jnp.broadcast_to(rows[d % 8:d % 8 + 1], (8, QB))

        def project(wqkv_v, wt_tail, h_v, acc_v, kt, *wt):
            blocks = [pl.ds(b * QB, QB) for b in range(NQ)]
            cp_x = [copy(x_hbm.at[rows], x_v.at[rows]) for rows in blocks]
            cp_tail = [copy(c_hbm, c_v.at[0]), mod_copy(DM, D - DM), mod_copy(D + DM, D - DM),
                       copy(wqkv_hbm.at[pl.ds(DM, D - DM)], wqkv_v.at[pl.ds(DM, D - DM)])]
            cp_mod = [mod_copy(0, DM), mod_copy(D, DM)]
            w_parts = [(pl.ds(0, DM), pl.ds(kind * D, D)) for kind in (1, 0, 2)]
            cp_w = [copy(wqkv_hbm.at[part_], wqkv_v.at[part_]) for part_ in w_parts]
            for cp in cp_x[:1] + cp_tail + cp_x[1:] + cp_w[:1] + cp_mod + cp_w[1:]:
                cp.start()

            def normalize(lo, n):
                h_v[pl.ds(lo, n), :] = _normalize_lanes(x_v[pl.ds(lo, n), :].astype(F32))

            def tail_pass(b, lo, hi, normalize_next):
                val = _dot_nt(wt_tail[lo:hi, :], h_v[blocks[b], DM:D] * ca1_tail + sa_tail)
                if normalize_next:
                    for k in range(16):
                        r = (hi - lo) // 8 * k // 18 * 8
                        pin(x_v, S, pltpu.bitcast(val[r:r + 8, 0:LANES], BF16))
                        normalize((b + 1) * QB + k * QB // 16, QB // 16)
                acc_v[lo:hi, blocks[b]] = val

            cp_x[0].wait()
            normalize(0, QB)
            for cp in cp_tail:
                cp.wait()
            sa_tail, ca1_tail = mod(DM, D - DM), 1.0 + mod(D + DM, D - DM)
            transpose(wqkv_v.at[pl.ds(DM, D - DM)], wt_tail)(0, D - DM)
            tail_pass(0, 0, D, False)
            for b in range(NQ - 1):
                cp_x[b + 1].wait()
                tail_pass(b, 0 if b else D, 3 * D, True)

            def transpose_w(kind, lo, n):
                wt[kind][:, pl.ds(pl.multiple_of(zero_s[0] + lo, LANES), n)] = (
                    wqkv_v[pl.ds(lo, n), pl.ds(kind * D, D)].T)

            def split_keys(c):
                tiles = [kt[pl.ds(t * LANES, LANES), pl.ds(c * KC, KC)].T for t in range(NT)]
                upper = lax.broadcasted_iota(I32, (KC, LANES), 1) >= LANES // 2
                tiles += [jnp.where(upper, tiles[t], tiles[t + 1]) for t in range(NT - 1)]
                for t, keys in enumerate(tiles):
                    kv[t, pl.ds(c * RV, RV), :] = keys[0:RV]
                    km[t, pl.ds(c * RM // 2, RM // 2), :] = pltpu.bitcast(keys[RV:KC].astype(BF16), I32)

            def first_keys(c):
                fill_head_keys(_key_tile(jnp.int32(0)), c * PIECES, PIECES)
                broadcast_keys(_key_tile(jnp.int32(0)), c, range(DH))
                for r in range(4 * DH * c, 4 * DH * (c + 1), 2 * DH):
                    ot[pl.ds(r, 8), :] = jnp.zeros((8, S), F32)

            def store_qkv(kind, i, cols, val):
                val = val + acc_v[pl.ds(kind * D + i * HALF, HALF), cols]
                if kind == 1:
                    kt[pl.ds(i * HALF, HALF), cols] = val
                    return
                low = lax.broadcasted_iota(I32, (8, QB), 0) < 4
                for u in range(0, HALF, 2 * DH):
                    v = [val[u + r:u + r + 8] for r in range(0, 2 * DH, 8)]
                    hd = (i * HALF + u) // DH
                    if kind == 0:
                        v = [r * QSCALE for r in v]
                        w = [pltpu.roll(r, 4, 0) for r in v[2:]]
                        qt[hd, :, cols] = jnp.concatenate([v[0], v[1], jnp.where(low, v[2], 0.0)], axis=0)
                        qt[hd + 1, :, cols] = jnp.concatenate(
                            [jnp.where(low, w[0], w[1]), jnp.where(low, w[1], w[2]), jnp.where(low, w[2], 0.0)], axis=0)
                    else:
                        vt[hd, :, cols] = jnp.concatenate([v[0], v[1], jnp.where(low, v[2], 1.0)], axis=0)
                        vt[hd + 1, :, cols] = jnp.concatenate([jnp.where(low, 1.0, v[2]), v[3], v[4]], axis=0)

            previous = []

            def main_pass(kind, b, jobs):
                left = [7]

                def multiply(lhs, rhs):
                    for _ in range(pl.cdiv(len(jobs), left[0])):
                        pin(kt, D, previous[0][0:8, 0:LANES])
                        jobs.pop(0)()
                    left[0] -= 1
                    previous[:] = [_dot_nt(lhs(), rhs())]
                    return previous[0]

                def h_block(k, t):
                    lanes = slice(k * DM // 2, (k + 1) * DM // 2)
                    return h_v[blocks[b + t], lanes] * ca1[:, lanes] + sa[:, lanes]

                _strassen(lambda i, k: wt[kind][pl.ds(i * HALF, HALF), pl.ds(k * DM // 2, DM // 2)], h_block,
                          ORDER_QKV, multiply, lambda i, t, val: store_qkv(kind, i, blocks[b + t], val))

            job = functools.partial
            cp_w[0].wait()
            transpose_w(1, 0, DM)
            tail_pass(NQ - 1, 0, 3 * D, False)
            for cp in cp_mod:
                cp.wait()
            sa, ca1 = mod(0, DM), 1.0 + mod(D, DM)
            main_pass(1, 0, [])
            cp_w[1].wait()
            cp_w[2].wait()
            for cp in late:
                cp.start()
            main_pass(1, 2, [job(transpose_w, kind, lo, LANES) for kind in (0, 2) for lo in range(0, DM, LANES)])
            main_pass(0, 0, [job(transpose(x_v, xt), lo, LANES) for lo in range(0, S, LANES)])
            main_pass(2, 0, [job(split_keys, c) for c in range(HC)]
                      + [job(broadcast_queries, 0, b, range(DH)) for b in range(2)])
            main_pass(2, 2, [job(split_keys, c) for c in range(HC, NCH)])
            main_pass(0, 2, [job(first_keys, c) for c in range(HC)])

        pl.run_scoped(project, pltpu.VMEM((D, 3 * D), BF16), pltpu.VMEM((3 * D, D - DM), BF16),
                      pltpu.VMEM((S, D), F32), pltpu.VMEM((3 * D, S), F32), pltpu.VMEM((D + 8, S), F32),
                      *[pltpu.VMEM((D, DM), BF16)] * 3)

        def step(n):
            half, rest = divmod(n % STEPS, NQ * HC)
            blk, c = divmod(rest, HC)
            return blk, half * HC + c

        def load_p(n, lo, rows):
            return ring[n % RING, pl.ds(8 * lo, 8 * rows), :]

        def accumulate(hd, blk, c, p, acc):
            o = _dot(vt[hd, :, pl.ds(c * KC, KC)], p)
            if c == HC:
                acc = part[zero_s[0] + blk]
            acc = o if c == 0 else o + acc
            if c == HC - 1:
                part[blk] = acc
            if c == NCH - 1:
                sums[blk] = acc
            return acc

        def store_output(hd, cols, acc):
            odd = hd & 1
            sub = lax.broadcasted_iota(I32, (8, LANES), 0)
            total = jnp.where(odd == 1, acc[0:1], acc[23:24])
            inv = pl.reciprocal(total, approx=True)
            o = acc * (inv * (2.0 - total * inv))
            r = pl.multiple_of(((hd * DH) >> 3) << 3, 8)
            ot[pl.ds(r, 8), cols] = jnp.where(sub < 4 * odd, ot[pl.ds(r, 8), cols], o[0:8])
            ot[pl.ds(pl.multiple_of(r + 8, 8), 16), cols] = o[8:24]
            return total

        def finish(hd, blk, u, unsafe):
            acc = sums[zero_s[0] + blk, :, pl.ds(u * LANES, LANES)]
            total = store_output(hd, pl.ds(blk * QB + u * LANES, LANES), acc)
            mag = jnp.abs(acc)
            ok = (mag[0:8] < ACC_HI) & (mag[8:16] < ACC_HI) & (mag[16:24] < ACC_HI) & (total > SUM_LO)
            return jnp.where(ok, unsafe, 1.0)

        def head(hd, acc, unsafe, p, last):
            z = zero_s[0]
            prv, nxt = jnp.maximum(hd - 1, 0), jnp.minimum(hd + 1, H - 1)
            keys = (_key_tile(hd), _key_tile(nxt))
            for n in range(STEPS):
                blk, c = step(n)
                half, rest = divmod(n, NQ * HC)
                lhs = pltpu.bitcast(kh[pl.ds(c * RM // 2, RM // 2), :], BF16)[:, 0:24]
                pm = jnp.exp2(_dot(lhs, qt[hd, :, pl.ds(blk * QB, QB)]))
                p_next = []
                d, r = 0, KC // 8
                for j in range(PIECES):
                    ring[n % RING, pl.ds(RV + 16 * j, 16), :] = pm[16 * j:16 * j + 16]
                    token = pm[16 * j:16 * j + 8, 0:LANES]
                    ring[z + RING, 0:8, 0:LANES] = token
                    bc[z + KB1, :, 0:LANES] = token
                    if P_LOADS[j]:
                        r -= P_LOADS[j]
                        p_next.insert(0, load_p(n - LAG + 1, r, P_LOADS[j]))
                    for _ in range((DIMS_LAST if last and n + 1 == STEPS else DIMS)[j]):
                        kk, qq = bc[key_slot(c, d)], bc[blk * DH + d]
                        prod = jnp.concatenate(
                            [_tile_lanes(kk[:, 0:LANES], QB) * qq, _tile_lanes(kk[:, LANES:], QB) * qq], axis=0)
                        scores = prod if d == 0 else scores + prod
                        d += 1
                    fill, k = divmod((n - 40) % STEPS, 12)
                    if fill < NQ:
                        dims = range((5 * k + 2) // 3, (5 * k + 7) // 3)
                        broadcast_queries(nxt if half else hd, fill, [e for e, at in zip(dims, Q_FILLS) if at == j])
                    if j in K_FILLS:
                        broadcast_keys(keys[half], (1 - half) * HC + rest // 4, [5 * (rest % 4) + K_FILLS.index(j)])
                    if j == 1 and rest < HC * PIECES // 4:
                        fill_head_keys(keys[half], (1 - half) * HC * PIECES + 4 * rest, 4)
                    if j == 0:
                        acc = accumulate(prv if n < LAG else hd, *step(n - LAG), p, acc)
                    if j == 0 and fill >= NQ:
                        sums[z + NQ, 0:8, 0:LANES] = token
                        unsafe = finish(prv, *divmod(n - 24, QTILES), unsafe)
                ring[n % RING, 0:RV, :] = jnp.exp2(scores)
                p = jnp.concatenate(p_next, axis=0)
            return acc, unsafe, p

        def trip(i, carry):
            carry = (*carry, load_p(-LAG, 0, KC // 8))
            for k in range(HEADS_PER_TRIP):
                carry = head(HEADS_PER_TRIP * i + k, *carry, k + 1 == HEADS_PER_TRIP)
            return carry[:2]

        for n in range(-LAG, 0):
            ring[n % RING] = jnp.zeros((KC, QB), F32)
        sums[...] = jnp.ones_like(sums)
        acc, unsafe = lax.fori_loop(0, H // HEADS_PER_TRIP, trip,
                                    (jnp.ones((24, QB), F32), jnp.zeros((8, LANES), F32)))
        for cp in late:
            cp.wait()
        transpose(wo_v, wot)(0, D)
        mod_v[...] = jnp.broadcast_to(mod(2 * D, 4 * D), mod_v.shape)
        for n in range(-LAG, 0):
            acc = accumulate(jnp.int32(H - 1), *step(n), load_p(n, 0, KC // 8), acc)
        for u in range(NQ * QTILES):
            unsafe = finish(jnp.int32(H - 1), *divmod(u, QTILES), unsafe)

        @pl.when(jnp.max(unsafe) > 0.0)
        def _():
            @pl.loop(0, H * S // LANES)
            def _(i):
                hd = i >> 4
                cols = pl.ds(pl.multiple_of((i & (S // LANES - 1)) * LANES, LANES), LANES)
                q = qt[hd, :, cols]
                t, off = _key_tile(hd)
                sm = _dot(pltpu.bitcast(_aligned_keys(km[t], off), BF16)[:, 0:24], q)
                sv = _dot(_aligned_keys(kv[t], off)[:, 0:24], q)
                top = jnp.maximum(jnp.max(sm, axis=0, keepdims=True), jnp.max(sv, axis=0, keepdims=True))
                pm, pv = jnp.exp2(sm - top), jnp.exp2(sv - top)
                p = [x for c in range(NCH) for x in (pv[c * RV:(c + 1) * RV], pm[c * RM:(c + 1) * RM])]
                store_output(hd, cols, _dot(vt[hd], jnp.concatenate(p, axis=0)))

    pl.run_scoped(
        attention_half,
        pltpu.VMEM((2 * NT - 1, NCH * RV, LANES), F32),
        pltpu.VMEM((2 * NT - 1, NCH * RM // 2, LANES), I32),
        pltpu.VMEM((NCH * RM // 2, LANES), I32),
        pltpu.VMEM((H, 24, S), F32),
        pltpu.VMEM((H, 24, S), F32),
        pltpu.VMEM((KB1 + 1, 8, QB), F32),
        pltpu.VMEM((RING + 1, KC, QB), F32),
        pltpu.VMEM((NQ, 24, QB), F32),
        pltpu.VMEM((NQ + 1, 24, QB), F32),
    )

    def ffn_half(x1, h2, act, out_v):
        wd_v[F:FP, :] = jnp.zeros((FP - F, D), BF16)
        act[F:FP, :] = jnp.zeros((FP - F, S), F32)
        ga, sb, cb1, gb = (
            jnp.concatenate([(one + mod_v[:, k * D:(k + 1) * D]) * scale] * (LANES // 8), axis=0).T
            for k, (one, scale) in enumerate(((0.0, 1.0), (0.0, GELU_IN), (1.0, GELU_IN), (0.0, 0.5 / GELU_IN ** 2))))
        jobs = []

        def multiply(lhs, rhs, per_product=0):
            lhs, rhs = lhs(), rhs()
            for _ in range(min(per_product, len(jobs))):
                jobs.pop(0)()
            return _dot(lhs, rhs)

        def normalize(tile):
            cols = pl.ds(tile * LANES, LANES)
            stats = []

            def mean():
                stats.append(_mean_rows(x1[:, cols]))

            def scale():
                d = x1[:, cols] - stats[0]
                stats.append(lax.rsqrt(_mean_rows(d * d) + EPS))

            def apply(rows):
                h2[rows, cols] = (x1[rows, cols] - stats[0]) * stats[1] * cb1[rows] + sb[rows]

            return [mean, scale, functools.partial(apply, slice(0, HALF)), functools.partial(apply, slice(HALF, D))]

        for b in range(0, NQ, 2):
            seen = set()

            def residual(i, t, val):
                rows, cols = slice(i * HALF, (i + 1) * HALF), pl.ds((b + t) * QB, QB)
                val = _dot(wot[rows, DM:D], ot[DM:D, cols]) + val
                x1[rows, cols] = xt[rows, cols].astype(F32) + _tile_lanes(ga[rows], QB) * val
                if t in seen:
                    for u in range(QTILES):
                        jobs.extend(normalize((b + t) * QTILES + u))
                seen.add(t)

            _strassen(lambda i, k: wot[pl.ds(i * HALF, HALF), pl.ds(k * DM // 2, DM // 2)],
                      lambda k, t: ot[pl.ds(k * DM // 2, DM // 2), pl.ds((b + t) * QB, QB)],
                      ORDER_PROJ, functools.partial(multiply, per_product=4), residual)

        def gated(lo, size, b, orders):
            n = 1 << len(orders)
            m = 2 * size // n
            other = {}

            def weights(i, lanes):
                rows = pl.ds(pl.multiple_of(lo, 64) + i % (n // 2) * m, m)
                return rows, (wg_v if i < n // 2 else wu_v)[rows, lanes]

            def activate(i, t, val):
                cols = pl.ds((b + t) * QB, QB)
                rows, w = weights(i, slice(DM, D))
                val = _dot(w, h2[DM:D, cols]) + val
                if i < n // 2:
                    val = _gelu_scaled(val)
                if (i % (n // 2), t) in other:
                    act[rows, cols] = other[i % (n // 2), t] * val
                other[i % (n // 2), t] = val

            _strassen(lambda i, k: weights(i, pl.ds(k * DM // n, DM // n))[1],
                      lambda k, t: h2[pl.ds(k * DM // n, DM // n), pl.ds((b + t) * QB, QB)],
                      orders, functools.partial(multiply, per_product=8), activate)

        gated(0, UP_FIRST, 0, ORDER_UP1)
        gated(0, UP_FIRST, 2, ORDER_UP1)

        @pl.loop(0, UP_CHUNKS)
        def _(chunk):
            n = pl.cdiv(FP // LANES, UP_CHUNKS)
            transpose(wd_v, wdt)(jnp.minimum(chunk * n, FP // LANES - n) * LANES, n * LANES)
            size = (F - UP_FIRST) // UP_CHUNKS
            gated(UP_FIRST + chunk * size, size, 0, ORDER_UP2)

        tail = {}
        _strassen(lambda i, k: wdt[pl.ds(i * HALF, HALF), pl.ds(FM + k * LANES, LANES)],
                  lambda k, t: act[pl.ds(FM + k * LANES, LANES), pl.ds(t * QB, QB)],
                  ORDER_TAIL, multiply, lambda i, t, val: tail.update({(i, t): val}))
        parts = [{} for _ in range(NQ)]
        writes, due = [], []

        def write(lo, y):
            cols = pl.ds(lo, y.shape[1])
            out_v[cols, :] = (x1[:, cols] + _tile_lanes(gb, y.shape[1]) * y).astype(out_v.dtype).T
            writes.append(copy(out_v.at[cols], out_hbm.at[cols]))
            writes[-1].start()

        def multiply_in_time(lhs, rhs):
            for entry in due:
                if entry[0] == 0:
                    rows = pl.ds(pl.multiple_of(zero_s[0] + entry[1], 16), 16)
                    pin(act, FP, pltpu.bitcast(out_v[rows, 0:LANES], F32))
                entry[0] -= 1
            return _dot(lhs(), rhs())

        def gather(i, t, val):
            if t < NQ // 2:
                val = val + tail[i // 2, t][i % 2 * D // 4:(i % 2 + 1) * D // 4]
            parts[t][i] = val
            if t < NQ // 2 and len(parts[t]) == 4:
                write(t * QB, jnp.concatenate([parts[t][k] for k in range(4)], axis=0))
                due.append([7, t * QB])

        _strassen(lambda i, k: wdt[pl.ds(i * D // 4, D // 4), pl.ds(k * FM // 4, FM // 4)],
                  lambda k, t: act[pl.ds(k * FM // 4, FM // 4), pl.ds(t * QB, QB)],
                  ORDER_DOWN, multiply_in_time, gather)
        for lo in range(S // 2, S, OUT_TAIL):
            y = jnp.concatenate([parts[lo // QB][k][:, lo % QB:lo % QB + OUT_TAIL] for k in range(4)], axis=0)
            write(lo, multiply_in_time(lambda: wdt[:, FM:FP], lambda: act[FM:FP, pl.ds(lo, OUT_TAIL)]) + y)
        for cp in writes:
            cp.wait()

    pl.run_scoped(ffn_half, pltpu.VMEM((D, S), F32), pltpu.VMEM((D, S), F32), pltpu.VMEM((FP + 8, S), F32),
                  pltpu.VMEM((S, D), out_hbm.dtype))


@jax.jit
def pallas_adaLN_cond__mha_block__geglu_ffn__prompt_kernel(
    A_x: jax.Array,
    A_wqkv: jax.Array,
    A_wo: jax.Array,
    B_x: jax.Array,
    B_w_gate: jax.Array,
    B_w_up: jax.Array,
    B_w_down: jax.Array,
    c: jax.Array,
    w_mod: jax.Array,
):
    del B_x
    hbm = pl.BlockSpec(memory_space=pltpu.HBM)
    out = pl.pallas_call(
        _kernel,
        out_shape=jax.ShapeDtypeStruct((S, D), A_x.dtype),
        in_specs=[hbm] * 8,
        out_specs=hbm,
        scratch_shapes=[
            pltpu.VMEM((32, 1, D), BF16),
            pltpu.VMEM((S + 64, D), BF16),
            pltpu.VMEM((D, D), BF16),
            pltpu.VMEM((F, D), BF16),
            pltpu.VMEM((F, D), BF16),
            pltpu.VMEM((FP, D), BF16),
            pltpu.VMEM((D, 6 * D), BF16),
            pltpu.VMEM((D, D), BF16),
            pltpu.VMEM((D, FP), BF16),
            pltpu.VMEM((D, S), BF16),
            pltpu.VMEM((D, S), F32),
            pltpu.VMEM((8, 4 * D), F32),
            pltpu.SMEM((2,), I32),
            pltpu.SemaphoreType.DMA((18 + NQ // 2 + S // 2 // OUT_TAIL,)),
        ],
        compiler_params=pltpu.CompilerParams(vmem_limit_bytes=126 * 1024 * 1024),
        name="adaln_block",
    )(A_x.reshape(S, D), A_wqkv, A_wo, B_w_gate.T, B_w_up.T, B_w_down, c, w_mod)
    return out.reshape(1, S, D)
```
